```python
import os as _os
_os.environ.setdefault("JAX_PLATFORMS", "cpu")
import jax
import jax.numpy as jnp

def _softmax(x, axis=-1):
    return jax.nn.softmax(x, axis=axis)
def _gelu(x):
    return jax.nn.gelu(x, approximate=True)
def _silu(x):
    return jax.nn.silu(x)
def _sigmoid(x):
    return jax.nn.sigmoid(x)
def _layernorm(x, axis=-1, eps=1e-5):
    m = jnp.mean(x, axis=axis, keepdims=True)
    v = jnp.var(x, axis=axis, keepdims=True)
    return (x - m) / jnp.sqrt(v + eps)
def _scatter_add(tgt, idx, src, axis=0):
    return tgt.at[idx].add(src)
def _segment_sum(src, seg, n):
    return jax.ops.segment_sum(src, seg, n)
class _Rng:
    def __init__(self, key):
        self._k = key
    def _next(self):
        self._k, sub = jax.random.split(self._k)
        return sub
    def normal(self, shape):
        return jax.random.normal(self._next(), shape, dtype=jnp.bfloat16)
    def randint(self, lo, hi, shape):
        return jax.random.randint(self._next(), shape, lo, hi, dtype=jnp.int32)
    def uniform(self, shape, lo=0.0, hi=1.0):
        return jax.random.uniform(self._next(), shape, jnp.bfloat16, lo, hi)
    def permutation(self, n):
        return jax.random.permutation(self._next(), n)


kernel_name = 'interleave_layers__sliding_local_dilated__softmax_full_mha__prompt'

def setup_inputs():
    _rng = _Rng(jax.random.key(int.from_bytes(__import__("os").urandom(4), "little")))
    _w = (lambda a: (lambda t: t.astype(jnp.bfloat16) if jnp.issubdtype(t.dtype, jnp.floating) else t)(jnp.asarray(a)))
    def _A_setup():
        B, S, D = 1, 2048, 512
        return {
            "x": _w((lambda *s: _rng.normal(s) * 0.05)(B, S, D)),
            "wqkv": _w((lambda *s: _rng.normal(s) * 0.05)(D, 3 * D)),
            "wo": _w((lambda *s: _rng.normal(s) * 0.05)(D, D)),
        }
    _A_in = _A_setup()

    def _B_setup():
        B, S, D = 1, 2048, 512
        return {
            "x": _w((lambda *s: _rng.normal(s) * 0.05)(B, S, D)),
            "wqkv": _w((lambda *s: _rng.normal(s) * 0.05)(D, 3 * D)),
            "wo": _w((lambda *s: _rng.normal(s) * 0.05)(D, D)),
        }
    _B_in = _B_setup()

    return {
        "A_x": _A_in["x"],
        "A_wqkv": _A_in["wqkv"],
        "A_wo": _A_in["wo"],
        "B_x": _B_in["x"],
        "B_wqkv": _B_in["wqkv"],
        "B_wo": _B_in["wo"],
    }

def reference(A_x, A_wqkv, A_wo, B_x, B_wqkv, B_wo):
    def _A_ref(x, wqkv, wo):
        B, S, D = x.shape
        H = 32; Dh = D // H
        W, dil = 8, 2
        qkv = (lambda x, *d: x.transpose(*d))((x @ wqkv).reshape(B, S, 3, H, Dh), 2, 0, 3, 1, 4)
        q, k, v = qkv[0], qkv[1], qkv[2]
        scale = Dh ** -0.5
        pos = jnp.arange(S)
        off = jnp.arange(W) * dil
        idx = pos[:, None] - off[None, :]
        mask = idx >= 0
        idx_c = jnp.where(mask, idx, 0).reshape(-1)
        kg = k[:, :, idx_c, :].reshape(B, H, S, W, Dh)
        vg = v[:, :, idx_c, :].reshape(B, H, S, W, Dh)
        logits = jnp.einsum("bhsd,bhswd->bhsw", q, kg) * scale
        logits = jnp.where(mask[None, None, :, :], logits, -1e9)
        attn = _softmax(logits, axis=-1)
        o = jnp.einsum("bhsw,bhswd->bhsd", attn, vg)
        return (lambda x, *d: x.transpose(*d))(o, 0, 2, 1, 3).reshape(B, S, D) @ wo

    def _B_ref(x, wqkv, wo):
        B, S, D = x.shape
        H = 32; Dh = D // H
        qkv = (lambda x, *d: x.transpose(*d))((x @ wqkv).reshape(B, S, 3, H, Dh), 2, 0, 3, 1, 4)
        q, k, v = qkv[0], qkv[1], qkv[2]
        scale = Dh ** -0.5
        scores = jnp.einsum("bhqd,bhkd->bhqk", q, k) * scale
        p = _softmax(scores, axis=-1)
        o = jnp.einsum("bhqk,bhkd->bhqd", p, v)
        return (lambda x, *d: x.transpose(*d))(o, 0, 2, 1, 3).reshape(B, S, D) @ wo

    x = A_x
    x = x + _A_ref(_layernorm(x, axis=-1), A_wqkv, A_wo)
    x = x + _B_ref(_layernorm(x, axis=-1), B_wqkv, B_wo)
    x = x + _A_ref(_layernorm(x, axis=-1), A_wqkv, A_wo)
    x = x + _B_ref(_layernorm(x, axis=-1), B_wqkv, B_wo)
    return x
```

```python
import math

import jax
import jax.numpy as jnp
from jax import lax
import jax.experimental.pallas as pl
import jax.experimental.pallas.tpu as pltpu

S, D, H, DH = 2048, 512, 32, 16
WIN, DIL = 8, 2
NG = H // 8
NCOL = S // 128
NR = NCOL // DIL
BACK = WIN - 1
LOG2E = math.log2(math.e)
QSCALE = DH ** -0.5 * LOG2E
EPS = 1e-5
TB = 512
L_MIN, L_MAX = 2.0 ** -40, 2.0 ** 60
OFF = 16
KM = 128 - OFF
NM, NV = NCOL * KM, NCOL * OFF
AHEAD = 160

F32, BF16, U32 = jnp.float32, jnp.bfloat16, jnp.uint32


def _dot(a, b):
    return jnp.dot(a, b, preferred_element_type=F32)


def _pack(x):
    return pltpu.bitcast(x.astype(BF16), U32)


def _unpack(x):
    return pltpu.bitcast(x, BF16)


def _layernorm_t(x):
    n = x.shape[1]
    mean = jnp.sum(jnp.sum(x.reshape(D // 8, 8, n), axis=0), axis=0, keepdims=True) * (1.0 / D)
    xc = x - mean
    var = jnp.sum(jnp.sum((xc * xc).reshape(D // 8, 8, n), axis=0), axis=0, keepdims=True) * (1.0 / D)
    return xc * lax.rsqrt(var + EPS), var


def _ds(start, size):
    return pl.ds(start if isinstance(start, int) else pl.multiple_of(start, size), size)


def _block_of(c):
    i = (c % DIL) * NR + c // DIL
    return slice(i * 128, (i + 1) * 128)


def _one_hot(source_of_row):
    r = lax.broadcasted_iota(jnp.int32, (128, 128), 0)
    c = lax.broadcasted_iota(jnp.int32, (128, 128), 1)
    return jnp.where(c == source_of_row(r), 1.0, 0.0).astype(BF16)


def _dot_nt(a, b):
    return lax.dot_general(a, b, (((1,), (1,)), ((), ())), preferred_element_type=F32)


def _kernel(x_hbm, wa_hbm, woa_hbm, wb_hbm, wob_hbm, out_hbm,
            x_st, wa_st, woa_st, wb_st, wob_st, sems,
            xt, x_mid, xn, wa, wb, wo, a_o, a_q0, a_k0, a_v0, a_q1, a_k1, a_v1,
            b_qf, b_q, b_v, b_km, b_kv, b_kb0, b_kb1, b_s, b_o, b_l):
    NF = D // 128

    def lane_block(f):
        return pl.ds(pl.multiple_of(f * 128, 128), 128)

    def x_copy(f):
        return pltpu.make_async_copy(x_hbm.at[:, lane_block(f)], x_st.at[f], sems.at[f])

    def out_copy(f, b):
        rows = pl.ds(b * 512, 512)
        return pltpu.make_async_copy(x_st.at[f, rows], out_hbm.at[rows, lane_block(f)], sems.at[4 * f + b])

    def a_copies(g):
        cols = [_ds((part * NG + g) * 128, 128) for part in range(3)]
        return [pltpu.make_async_copy(wa_hbm.at[:, c], wa_st.at[:, c], sems.at[NF + 4 * g + n])
                for n, c in enumerate(cols)] + [pltpu.make_async_copy(
                    woa_hbm.at[_ds(g * 128, 128)], woa_st.at[_ds(g * 128, 128)], sems.at[NF + 4 * g + 3])]

    b_copies = [pltpu.make_async_copy(src, dst, sems.at[NF + 4 * NG + i])
                for i, (src, dst) in enumerate([(wb_hbm, wb_st), (wob_hbm, wob_st)])]

    def split16(r):
        return (r % 8) * 16 + r // 8

    def merge16(r):
        return (r % 16) * 8 + r // 16

    def transpose_qkv(w_st, w, select, g):
        for part in range(3):
            w[g, part * 64:(part + 1) * 64, :] = _pack(
                _dot_nt(select, w_st[:, _ds((part * NG + g) * 128, 128)]))

    def load_inputs():
        x_copy(0).start()
        x_copy(1).start()

        def x_block(f, carry):
            x_copy(f).wait()
            pl.when(f + 2 < NF)(lambda: x_copy(jnp.minimum(f + 2, NF - 1)).start())

            @pl.when(f + 2 >= NF)
            def _():
                for cp in a_copies(jnp.maximum(f + 2 - NF, 0)):
                    cp.start()

            perm = _one_hot(split16)
            n = 4
            for c0 in range(0, NCOL, n):
                ys = [_dot(perm[c0 * 8:(c0 + n) * 8], jnp.concatenate(
                    [x_st[f, (4 * b + i) * 128:(4 * b + i + 1) * 128, :] for i in range(4)], axis=1))
                    for b in range(NCOL // 4)]
                for c in range(n):
                    tile = jnp.concatenate([y[c * 8:(c + 1) * 8, i * 128:(i + 1) * 128]
                                            for y in ys for i in range(4)], axis=0)
                    xt[lane_block(f), _block_of(c0 + c)] = tile.T
            return carry

        lax.fori_loop(0, NF, x_block, 0)

        def norm_and_weights(g, carry):
            for cp in a_copies(g):
                cp.wait()

            @pl.when(g + 2 < NG)
            def _():
                for cp in a_copies(jnp.minimum(g + 2, NG - 1)):
                    cp.start()

            perm = _one_hot(split16)
            transpose_qkv(wa_st, wa, perm, g)
            wo[0, :, lane_block(g)] = _pack(_dot(perm, woa_st[lane_block(g), :]).T)
            for j in range(2):
                cols = _ds(g * TB + j * (TB // 2), TB // 2)
                xn[:, cols] = _pack(_layernorm_t(xt[:, cols])[0])
            return carry

        lax.fori_loop(0, NG, norm_and_weights, 0)
        for cp in b_copies:
            cp.start()

    def load_b_weights():
        for cp in b_copies:
            cp.wait()
        eye = _one_hot(lambda r: r)
        for g in range(NG):
            rows = slice(g * 128, (g + 1) * 128)
            wo[1, :, rows] = _pack(wob_st[rows, :].astype(F32).T)
            if g < NG // 2:
                for part in range(3):
                    col = (part * NG + g) * 128
                    wb[g, part * 64:(part + 1) * 64, :] = _pack(wb_st[:, col:col + 128].astype(F32).T)
            else:
                transpose_qkv(wb_st, wb, eye, g)

    def store_output():
        def block(f, carry):
            perm = _one_hot(merge16)
            tiles = [xt[lane_block(f), _block_of(c)].T for c in range(NCOL)]
            for b in range(NCOL // 4):
                y = jnp.concatenate(
                    [jnp.concatenate([t[(4 * b + i) * 8:(4 * b + i + 1) * 8] for t in tiles], axis=0)
                     for i in range(4)], axis=1)
                y = _dot(perm, y.astype(BF16)).astype(BF16)
                for i in range(4):
                    x_st[f, (4 * b + i) * 128:(4 * b + i + 1) * 128, :] = y[:, i * 128:(i + 1) * 128]
                out_copy(f, b).start()
            return carry

        lax.fori_loop(0, NF, block, 0)
        for f in range(NF):
            for b in range(NCOL // 4):
                out_copy(f, b).wait()

    a_bufs = [(a_q0, a_k0, a_v0), (a_q1, a_k1, a_v1)]

    def a_attend(stage, slot, i):
        res, g = stage // NG, stage % NG
        a_q, a_k, a_v = a_bufs[slot]
        first_lane = lax.broadcasted_iota(jnp.int32, (8, 128), 1) == 0
        logits = []
        for w in range(WIN):
            lg = jnp.sum((a_q[BACK + i] * a_k[BACK + i - w]).reshape(DH, 8, 128), axis=0) * QSCALE
            logits.append(jnp.where(first_lane, -1e9 * LOG2E, lg) if w > i else lg)
        m = logits[0]
        for lg in logits[1:]:
            m = jnp.maximum(m, lg)
        e = [jnp.exp2(lg - m) for lg in logits]
        l = e[0]
        for y in e[1:]:
            l = l + y
        inv = 1.0 / l
        out = None
        for w in range(WIN):
            pr = (e[w] * inv)[None] * a_v[BACK + i - w].reshape(DH, 8, 128)
            out = pr if out is None else out + pr
        a_o[g, :, _ds((res * NR + i) * 128, 128)] = _pack(out.reshape(128, 128))

    def a_project(stage, slot, order):
        res, g = stage // NG, stage % NG
        first_lane = lax.broadcasted_iota(jnp.int32, (128, 128), 1) == 0
        jobs = [(part, a_bufs[slot][part], t) for part in order for t in range(NR * 128 // TB)]
        for part, ref, t in jobs:
            cols = _ds(res * NR * 128 + t * TB, TB)
            r = _dot(_unpack(wa[g, part * 64:(part + 1) * 64, :]), _unpack(xn[:, cols]))
            for j in range(TB // 128):
                i = t * (TB // 128) + j
                y = r[:, j * 128:(j + 1) * 128]
                ref[BACK + i] = y
                if i == 0:
                    first = jnp.broadcast_to(y[:, 0:1], (128, 128))
                if part and i >= NR - BACK:
                    y = pltpu.roll(y, 1, 1)
                    if part == 2:
                        y = jnp.where(first_lane, first, y)
                    ref[i - (NR - BACK)] = y

    def add_and_norm(x_in, x_out, wo, a, cols):
        x = x_in[:, cols] + _dot(_unpack(wo), a)
        x_out[:, cols] = x
        y, var = _layernorm_t(x)
        xn[:, cols] = _pack(y)
        return var

    def layer_a():
        def attend(n, slot):
            for i in range(NR):
                a_attend(n, slot, i)

        def two_stages(i, carry):
            attend(2 * i, 0)
            a_project(2 * i + 1, 1, (1, 0, 2))
            attend(2 * i + 1, 1)
            a_project(2 * i + 2, 0, (0, 1, 2))
            return carry

        last = DIL * NG - 1
        a_project(0, 0, (1, 2, 0))
        lax.fori_loop(0, last // 2, two_stages, 0)
        attend(last - 1, 0)
        a_project(last, 1, (1, 0, 2))
        attend(last, 1)
        add_and_norm(xt, x_mid, wo[0], _unpack(a_o[...].reshape(D // 2, S)), slice(0, S))

    def b_project(i, carry):
        g = NG - 1 - i
        heads = pl.ds(g * 8, 8)
        for t in range(S // TB):
            cols = slice(t * TB, (t + 1) * TB)
            k = _dot(_unpack(wb[g, 64:128, :]), _unpack(xn[:, cols]))
            for i in range(TB // 128):
                c = t * (TB // 128) + i
                kt = k[:, i * 128:(i + 1) * 128].T
                if c == 0:
                    mean = jnp.sum(jnp.sum(kt.reshape(16, 8, 128), axis=0), axis=0, keepdims=True) * (1.0 / 128)
                kt = kt - mean
                km, kv = _pack(kt[:KM]), kt[KM:]
                for j in range(8):
                    sh = (128 - DH * j) % 128
                    b_km[g * 8 + j, c * KM // 2:(c + 1) * KM // 2, :] = pltpu.roll(km, sh, 1) if j else km
                    b_kv[g * 8 + j, c * OFF:(c + 1) * OFF, :] = pltpu.roll(kv, sh, 1) if j else kv
        for t in range(S // TB):
            cols = slice(t * TB, (t + 1) * TB)
            r = _dot(_unpack(jnp.concatenate([wb[g, :64, :], wb[g, 128:, :]], axis=0)), _unpack(xn[:, cols]))
            q, v = r[:128], r[128:]
            q = q * QSCALE
            b_qf[heads, :, cols] = q.reshape(8, DH, TB)
            b_q[heads, :, cols] = _pack(q).reshape(8, 8, TB)
            b_v[heads, :, cols] = _pack(v).reshape(8, 8, TB)
        for j in range(DH * NV // 8):
            spread_key(g * 8, b_kb0, j)
        return carry

    def spread_key(h, kb_ref, i):
        d, r = divmod(i, NV // 8)
        kv = b_kv[h, r * 8:(r + 1) * 8, :]
        kb_ref[d, r * 8:(r + 1) * 8, :] = jnp.broadcast_to(kv[:, d:d + 1], (8, 128))

    def mxu_scores(h, u, k0, n):
        return _dot(_unpack(b_km[h, k0 // 2:(k0 + n) // 2, :])[:, :DH],
                    _unpack(b_q[h, :, u * TB:(u + 1) * TB]))

    def b_head_pair(i, carry):
        NT, NB = TB // 128, S // TB
        heads = [2 * i, 2 * i + 1, jnp.minimum(2 * i + 2, H - 1)]
        kbs = [b_kb0, b_kb1, b_kb0]
        spare = pl.multiple_of(jnp.minimum(i, 0) + NV, 8)
        units = [(g, t0, d) for g in range(NV // 16) for d in range(DH) for t0 in range(0, NT, 2)]
        n = NM // 16
        pieces = [(e, u, units[x * len(units) // n:(x + 1) * len(units) // n])
                  for e in range(2) for u in range(NB) for x in range(n)]
        per_head = len(pieces) // 2
        nspread = DH * NV // 8
        rows = [b_s[r * 8:(r + 1) * 8, :] for r in range(AHEAD // 8)]
        done, used, j, acc, pv = AHEAD, 0, 0, {}, {}
        for step in range(2 * NB * NCOL):
            e, hs = divmod(step, NB * NCOL)
            u, c = divmod(hs, NCOL)
            while done < used + KM + AHEAD:
                item, k0 = divmod(done, NM)
                n = min(used + KM + AHEAD - done, NM - k0)
                s = mxu_scores(heads[item // NB], item % NB, k0, n)
                rows += [s[r * 8:(r + 1) * 8] for r in range(n // 8)]
                done += n
            j0 = j
            while j < (used + KM) // 16:
                pe, pu, work = pieces[j]
                kb_ref = kbs[pe]
                fi = 2 * j - 4
                if j - j0 == 2 and step - 2 in pv:
                    kb_ref[0, pl.ds(spare, 8), :] = pv.pop(step - 2)[:8, :128]
                if AHEAD // 8 <= fi < len(rows):
                    kb_ref[0, pl.ds(spare, 8), :] = rows[fi][:, :128]
                lo, hi = [min(nspread, max(0, x - 8) * nspread * 64 // (44 * per_head))
                          for x in (j % per_head, j % per_head + 1)]
                if lo < hi and fi < len(rows) and j % 2 == 1:
                    b_kv[0, pl.ds(spare, 8), :] = rows[fi][:, :128]
                for x in range(lo, hi):
                    spread_key(heads[pe + 1], kbs[pe + 1], x)
                for g, t0, d in work:
                    kb = [kb_ref[d, g * 16 + r * 8:g * 16 + (r + 1) * 8, :] for r in range(2)]
                    for t in range(t0, t0 + 2):
                        q0 = pu * TB + t * 128
                        qb = jnp.broadcast_to(b_qf[heads[pe], d:d + 1, q0:q0 + 128], (8, 128))
                        for r in range(2):
                            key = (pe, pu, 2 * g + r, t)
                            acc[key] = acc[key] + kb[r] * qb if d else kb[r] * qb
                j += 1
            sv = [jnp.concatenate([acc.pop((e, u, r, t)) for t in range(NT)], axis=1)
                  for r in range(c * OFF // 8, (c + 1) * OFF // 8)]
            p = jnp.exp2(jnp.concatenate(rows[used // 8:(used + KM) // 8] + sv, axis=0))
            used += KM
            ll = jnp.sum(p.reshape(16, 8, TB), axis=0)
            pv[step] = oo = _dot(_unpack(b_v[heads[e], :, c * 128:(c + 1) * 128]), p.astype(BF16))
            l8, o = (ll, oo) if c == 0 else (l8 + ll, o + oo)
            if c == NCOL - 1:
                b_o[heads[e], :, u * TB:(u + 1) * TB] = o
                b_l[heads[e], :, u * TB:(u + 1) * TB] = l8
        b_s[...] = jnp.concatenate(rows[used // 8:], axis=0)
        return carry

    def b_exact_head(h, carry):
        wk = _unpack(wb[h // 8, pl.ds(pl.multiple_of(64 + (h % 8) * 8, 8), 8), :])
        k = _dot(wk, _unpack(xn[...])).astype(BF16)
        v = _unpack(b_v[h])

        def block(t, carry):
            cols = pl.ds(pl.multiple_of(t * 128, 128), 128)
            s = lax.dot_general(k, _unpack(b_q[h, :, cols]), (((0,), (0,)), ((), ())),
                                preferred_element_type=F32)
            p = jnp.exp2(s - jnp.max(s, axis=0, keepdims=True))
            l = jnp.sum(p, axis=0, keepdims=True)
            b_o[h, :, cols] = _dot(v, (p / l).astype(BF16))
            b_l[h, :, cols] = jnp.full((8, 128), 0.125, F32)
            return carry

        return lax.fori_loop(0, NCOL, block, carry)

    def b_heads_out(cols):
        l = jnp.sum(b_l[:, :, cols], axis=1, keepdims=True)
        a = b_o[:, :, cols] * (1.0 / l)
        return a.reshape(D, a.shape[2]).astype(BF16), l

    def layer_b():
        lax.fori_loop(0, NG, b_project, 0)
        b_s[...] = mxu_scores(0, 0, 0, AHEAD)
        lax.fori_loop(0, H // 2, b_head_pair, 0)

        ok = None
        for t in range(2):
            cols = slice(t * S // 2, (t + 1) * S // 2)
            a, l = b_heads_out(cols)
            var = add_and_norm(x_mid, xt, wo[1], a, cols)
            ok_t = jnp.where((jnp.min(l, axis=0) >= L_MIN) & (jnp.max(l, axis=0) <= L_MAX)
                             & (var < jnp.inf), 1.0, 0.0)
            ok = ok_t if t == 0 else jnp.minimum(ok, ok_t)

        @pl.when(jnp.min(ok) < 1.0)
        def _():
            def restore_input(t, carry):
                cols = lane_block(t)
                xn[:, cols] = _pack(_layernorm_t(x_mid[:, cols])[0])
                return carry

            lax.fori_loop(0, NCOL, restore_input, 0)
            lax.fori_loop(0, H, b_exact_head, 0)

            def block(t, carry):
                cols = lane_block(t)
                add_and_norm(x_mid, xt, wo[1], b_heads_out(cols)[0], cols)
                return carry

            lax.fori_loop(0, NCOL, block, 0)

    def layer_pair(i, carry):
        layer_a()
        pl.when(i == 0)(load_b_weights)
        layer_b()
        return carry

    load_inputs()
    lax.fori_loop(0, 2, layer_pair, 0)
    store_output()


@jax.jit
def pallas_interleave_layers__sliding_local_dilated__softmax_full_mha__prompt_kernel(
    A_x: jax.Array,
    A_wqkv: jax.Array,
    A_wo: jax.Array,
    B_x: jax.Array,
    B_wqkv: jax.Array,
    B_wo: jax.Array,
):
    del B_x
    assert A_x.shape == (1, S, D)
    vmem = pltpu.VMEM
    a_bufs = [vmem((BACK + NR, 128, 128), F32)] * 3
    out = pl.pallas_call(
        _kernel,
        out_shape=jax.ShapeDtypeStruct((S, D), BF16),
        in_specs=[pl.BlockSpec(memory_space=pl.ANY)] * 5,
        out_specs=pl.BlockSpec(memory_space=pl.ANY),
        scratch_shapes=[
            vmem((D // 128, S, 128), BF16), vmem((D, 3 * D), BF16), vmem((D, D), BF16),
            vmem((D, 3 * D), BF16), vmem((D, D), BF16), pltpu.SemaphoreType.DMA((D // 128 + 4 * NG + 2,)),
            vmem((D, S), F32), vmem((D, S), F32), vmem((D // 2, S), U32),
            vmem((NG, 192, D), U32), vmem((NG, 192, D), U32), vmem((2, D // 2, D), U32),
            vmem((NG, 64, S), U32), *a_bufs, *a_bufs,
            vmem((H, DH, S), F32), vmem((H, 8, S), U32), vmem((H, 8, S), U32),
            vmem((H, NM // 2, 128), U32), vmem((H, NV + 8, 128), F32),
            vmem((DH, NV + 8, 128), F32), vmem((DH, NV + 8, 128), F32), vmem((AHEAD, TB), F32),
            vmem((H, DH, S), F32), vmem((H, 8, S), F32),
        ],
        compiler_params=pltpu.CompilerParams(vmem_limit_bytes=100 * 2 ** 20),
    )(A_x.reshape(S, D).astype(BF16), A_wqkv.astype(BF16), A_wo.astype(BF16),
      B_wqkv.astype(BF16), B_wo.astype(BF16))
    return out.reshape(1, S, D)
```
